```python
import jax
import jax.numpy as jnp

def _softmax(x, axis=-1):
    return jax.nn.softmax(x, axis=axis)

def _gelu(x):
    return jax.nn.gelu(x, approximate=True)

def _silu(x):
    return jax.nn.silu(x)

def _sigmoid(x):
    return jax.nn.sigmoid(x)

def _layernorm(x, axis=-1, eps=1e-05):
    m = jnp.mean(x, axis=axis, keepdims=True)
    v = jnp.var(x, axis=axis, keepdims=True)
    return (x - m) / jnp.sqrt(v + eps)

def _scatter_add(tgt, idx, src, axis=0):
    return tgt.at[idx].add(src)

def _segment_sum(src, seg, n):
    return jax.ops.segment_sum(src, seg, n)

class _Rng:

    def __init__(self, key):
        self._k = key

    def _next(self):
        self._k, sub = jax.random.split(self._k)
        return sub

    def normal(self, shape):
        return jax.random.normal(self._next(), shape, dtype=jnp.bfloat16)

    def randint(self, lo, hi, shape):
        return jax.random.randint(self._next(), shape, lo, hi, dtype=jnp.int32)

    def uniform(self, shape, lo=0.0, hi=1.0):
        return jax.random.uniform(self._next(), shape, jnp.bfloat16, lo, hi)

    def permutation(self, n):
        return jax.random.permutation(self._next(), n)
kernel_name = 'adaLN_cond__grouped_kv_mqa__dense_activation_silu__prompt'

def _fwd_setup_inputs():
    _rng = _Rng(jax.random.key(int.from_bytes(__import__("os").urandom(4), "little")))
    _w = lambda a: (lambda t: t.astype(jnp.bfloat16) if jnp.issubdtype(t.dtype, jnp.floating) else t)(jnp.asarray(a))

    def _A_setup():
        B, S, D, H = (1, 2048, 640, 32)
        Dh = D // H
        return {'x': _w((lambda *s: _rng.normal(s) * 0.05)(B, S, D)), 'wq': _w((lambda *s: _rng.normal(s) * 0.05)(D, H * Dh)), 'wk': _w((lambda *s: _rng.normal(s) * 0.05)(D, Dh)), 'wv': _w((lambda *s: _rng.normal(s) * 0.05)(D, Dh)), 'wo': _w((lambda *s: _rng.normal(s) * 0.05)(H * Dh, D))}
    _A_in = _A_setup()

    def _B_setup():
        B, S, D, F = (1, 2048, 640, 1728)
        return {'x': _w((lambda *s: _rng.normal(s) * 0.05)(B, S, D)), 'w1': _w((lambda *s: _rng.normal(s) * 0.05)(D, F) * D ** (-0.5)), 'w2': _w((lambda *s: _rng.normal(s) * 0.05)(F, D) * F ** (-0.5))}
    _B_in = _B_setup()
    return {'A_x': _A_in['x'], 'A_wq': _A_in['wq'], 'A_wk': _A_in['wk'], 'A_wv': _A_in['wv'], 'A_wo': _A_in['wo'], 'B_x': _B_in['x'], 'B_w1': _B_in['w1'], 'B_w2': _B_in['w2'], 'c': _w((lambda *s: _rng.normal(s) * 0.05)(1, 640)), 'w_mod': _w((lambda *s: _rng.normal(s) * 0.05)(640, 6 * 640) * 640 ** (-0.5))}

def _fwd_reference(A_x, A_wq, A_wk, A_wv, A_wo, B_x, B_w1, B_w2, c, w_mod):

    def _A_ref(x, wq, wk, wv, wo):
        B, S, D = x.shape
        H = 32
        Dh = D // H
        q = (lambda x, *d: x.transpose(*d))((x @ wq).reshape(B, S, H, Dh), 0, 2, 1, 3)
        k = x @ wk
        v = x @ wv
        scores = jnp.einsum('bhqd,bkd->bhqk', q, k) * Dh ** (-0.5)
        p = _softmax(scores, axis=-1)
        o = jnp.einsum('bhqk,bkd->bhqd', p, v)
        return (lambda x, *d: x.transpose(*d))(o, 0, 2, 1, 3).reshape(B, S, H * Dh) @ wo

    def _B_ref(x, w1, w2):
        h = jnp.einsum('bsd,df->bsf', x, w1)
        h = _silu(h)
        out = jnp.einsum('bsf,fd->bsd', h, w2)
        return out
    x = A_x
    mod = (_silu(c) @ w_mod).reshape(c.shape[0], 6, 1, -1)
    sa, ca, ga, sb, cb, gb = (mod[:, 0].copy(), mod[:, 1].copy(), mod[:, 2].copy(), mod[:, 3].copy(), mod[:, 4].copy(), mod[:, 5].copy())
    h = _layernorm(x, axis=-1) * (1 + ca) + sa
    x = x + ga * _A_ref(h, A_wq, A_wk, A_wv, A_wo)
    h = _layernorm(x, axis=-1) * (1 + cb) + sb
    x = x + gb * _B_ref(h, B_w1, B_w2)
    return x

def setup_inputs():
    _inp = _fwd_setup_inputs()
    _gk = jax.random.fold_in(jax.random.key(int.from_bytes(__import__("os").urandom(4), "little")), 2 ** 31 - 1)
    _shapes = [[1, 2048, 640]]
    _dtypes = ['bfloat16']
    _gks = jax.random.split(_gk, len(_shapes))
    _gs = [jax.random.normal(k, s, dtype=jnp.dtype(d)) * 0.05 for k, s, d in zip(_gks, _shapes, _dtypes)]
    _inp['grad_out'] = _gs[0]
    return _inp

def reference(A_x, A_wq, A_wk, A_wv, A_wo, B_w1, B_w2, c, w_mod, B_x, grad_out):
    _const = dict(B_x=B_x)

    def _f(*_d):
        return _fwd_reference(**{'A_x': _d[0], 'A_wq': _d[1], 'A_wk': _d[2], 'A_wv': _d[3], 'A_wo': _d[4], 'B_w1': _d[5], 'B_w2': _d[6], 'c': _d[7], 'w_mod': _d[8], **_const})
    _out, _vjp = jax.vjp(_f, A_x, A_wq, A_wk, A_wv, A_wo, B_w1, B_w2, c, w_mod)
    _grads = _vjp(grad_out)
    _out0 = jnp.asarray(_out)
    return (_out0, *[jnp.asarray(_g) for _g in _grads])
```

```python
import math

import jax
import jax.numpy as jnp
from jax import lax
import jax.experimental.pallas as pl
import jax.experimental.pallas.tpu as pltpu

S, D, H, DH, F = 2048, 640, 32, 20, 1728
BQ = 512
NB = S // BQ
NL = BQ // 128
NP = H // 2
KC = 128
NC = S // KC
W = 24
FC = 192
EPS = 1e-5
SCALE = DH ** -0.5
LOG2E = math.log2(math.e)
LN2 = math.log(2.0)

BF, F32 = jnp.bfloat16, jnp.float32
_NN = (((1,), (0,)), ((), ()))
_NT = (((1,), (1,)), ((), ()))
_TN = (((0,), (0,)), ((), ()))


def _dot(a, b, dims=_NN):
    return lax.dot_general(a, b, dims, preferred_element_type=F32)


def _rows(shape):
    return lax.broadcasted_iota(jnp.int32, shape, 0)


def _rbf(x):
    return x.astype(BF).astype(F32)


def _wide(col):
    return jnp.concatenate([col] * NL, axis=1)


def _fold(x):
    acc = x[:, :128]
    for j in range(1, NL):
        acc = acc + x[:, j * 128:(j + 1) * 128]
    return acc


def _to_col(row):
    return jnp.broadcast_to(row, (128, D)).T


def _to_row(part):
    return jnp.sum(part.T, axis=0, keepdims=True)


def _feat_mean(x):
    return jnp.sum(x, axis=0, keepdims=True) * (1.0 / D)


def _normalize(x):
    xc = x - _feat_mean(x)
    rstd = lax.rsqrt(_feat_mean(xc * xc) + EPS)
    return xc * rstd, rstd


def _normalize_bwd(dn, n, rstd):
    return rstd * (dn - _feat_mean(dn) - n * _feat_mean(dn * n))


def _head(ref, pair, odd):
    if odd:
        w = pltpu.roll(ref[pair, 2 * DH - W:, :], DH, 0)
    else:
        w = ref[pair, :W, :]
    return jnp.where(_rows((W, BQ)) < DH, w, 0.0)


def _store_pair(ref, pair, even, odd):
    odd = pltpu.roll(odd, W - DH, 0)
    ref[pair, :16, :] = even[:16]
    ref[pair, 16:24, :] = jnp.where(_rows((8, BQ)) < 4, even[16:], odd[:8])
    ref[pair, 24:, :] = odd[8:]


def _as_weights(w):
    return jnp.concatenate([w, jnp.zeros((32 - W, BQ), F32)], axis=0).astype(BF)


def _kernel(x_hbm, wq_hbm, wkt_hbm, wvt_hbm, wo_hbm, w1t_hbm, w2_hbm, c_hbm, wmod_hbm, g_hbm,
            out_hbm, dx_hbm, dwq_hbm, dwkt_hbm, dwvt_hbm, dwo_hbm, dw1t_hbm, dw2_hbm, dc_hbm, dwmod_hbm,
            xt_ref, q_ref, dx1_ref, k_ref, v_ref, kt_ref, vt_ref, dkt_ref, dvt_ref,
            wq_ref, wkv_ref, wo_ref, w1t_ref, w2_ref, c_ref, mod_ref, dmod_ref,
            dwo_ref, dw1t_ref, dw2_ref, gin_ref, sem):
    def copy(src, dst, i):
        return pltpu.make_async_copy(src, dst, sem.at[i])

    def g_copy(b):
        return copy(g_hbm.at[pl.ds(pl.multiple_of(b * BQ, BQ), BQ)], gin_ref, 0)

    late = [copy(wo_hbm, wo_ref, 1), copy(w1t_hbm, w1t_ref, 2), copy(w2_hbm, w2_ref, 3)]

    def silu_c():
        c = c_ref[...].astype(F32)
        sig = jax.nn.sigmoid(c)
        return c, sig, _rbf(c * sig)

    def prologue(xin_ref, wmod_ref, wk_ref, wv_ref, wkvf_ref):
        def x_copy(b):
            rows = pl.ds(pl.multiple_of(b * BQ, BQ), BQ)
            return copy(x_hbm.at[rows], xin_ref.at[b], 4 + b)

        first = [copy(c_hbm, c_ref, 8),
                 copy(wmod_hbm.at[:, :2 * D], wmod_ref.at[:, :2 * D], 9),
                 copy(wkt_hbm, wk_ref, 10), copy(wvt_hbm, wv_ref, 11),
                 copy(wq_hbm, wq_ref, 12)]
        mod_rest = copy(wmod_hbm.at[:, 2 * D:], wmod_ref.at[:, 2 * D:], 13)
        for cp in first:
            cp.start()
        x_copy(0).start()

        for ref in (dwo_ref, dw1t_ref, dw2_ref, dmod_ref, dkt_ref, dvt_ref, wkvf_ref):
            ref[...] = jnp.zeros(ref.shape, F32)

        for cp in first:
            cp.wait()
        for b in range(1, NB):
            x_copy(b).start()
        mod_rest.start()

        sc = jnp.broadcast_to(silu_c()[2], (8, D))

        def modulation(j):
            m = _dot(sc, wmod_ref[:, j * D:(j + 1) * D])[:1]
            mod_ref[j] = _to_col(m + 1.0 if j in (1, 4) else m)

        modulation(0)
        modulation(1)
        wkvf_ref[:DH, :] = wk_ref[...].astype(F32)
        wkvf_ref[W:W + DH, :] = wv_ref[...].astype(F32)
        wkv_ref[...] = wkvf_ref[...].astype(BF)

        def block(b, carry):
            x_copy(b).wait()
            xt = xin_ref[b].astype(F32).T
            xt_ref[b] = xt.astype(BF)
            n1, _ = _normalize(xt)
            h1 = (n1 * _wide(mod_ref[1]) + _wide(mod_ref[0])).astype(BF)
            kv = _rbf(_dot(wkv_ref[...], h1))
            r = _rows((W, BQ))
            kt = kv[:W]
            vt = jnp.where((r >= DH) & (r < DH + 3), 1.0, kv[W:])
            cols = pl.ds(pl.multiple_of(b * BQ, BQ), BQ)
            kt_ref[:, cols] = kt
            vt_ref[:, cols] = vt
            pad = jnp.zeros((128 - W, BQ), F32)
            k_ref[cols, :] = jnp.concatenate([kt, pad], axis=0).T.astype(BF)
            v_ref[cols, :] = jnp.concatenate([vt, pad], axis=0).T.astype(BF)
            qt = _rbf(_dot(wq_ref[...], h1, _TN) * (SCALE * LOG2E))
            q_ref[pl.ds(b * NP, NP)] = qt.reshape(NP, 2 * DH, BQ)
            return carry

        lax.fori_loop(0, NB, block, 0)
        mod_rest.wait()
        g_copy(0).start()
        for cp in late:
            cp.start()
        for j in range(2, 6):
            modulation(j)

    pl.run_scoped(prologue,
                  pltpu.VMEM((NB, BQ, D), BF), pltpu.VMEM((D, 6 * D), BF),
                  pltpu.VMEM((DH, D), BF), pltpu.VMEM((DH, D), BF), pltpu.VMEM((2 * W, D), F32))

    early_out = [copy(wo_ref, dwo_hbm, 1), copy(w1t_ref, dw1t_hbm, 2), copy(w2_ref, dw2_hbm, 3)]

    def main(p_ref, s_ref, m_ref, linv_ref, o_ref, do_ref, act_ref, dact_ref, ost_ref):
        def out_copy(b):
            return copy(ost_ref, out_hbm.at[pl.ds(pl.multiple_of(b * BQ, BQ), BQ)], 4)

        def keys(c):
            return slice(c * KC, (c + 1) * KC)

        def load_p(h, c, dtype):
            return jnp.concatenate(
                [p_ref[h, j, keys(c), :].astype(dtype) for j in range(NL)], axis=1)

        def scores(q, c, mx):
            s = _dot(k_ref[keys(c), :32], q)
            s_ref[keys(c), :] = s
            part = jnp.max(s.reshape(KC // 8, 8, BQ), axis=0)
            return part if mx is None else jnp.maximum(mx, part)

        def row_max(mx):
            return jnp.broadcast_to(jnp.max(mx, axis=0, keepdims=True), (8, BQ))

        mx = None
        q0 = _as_weights(_head(q_ref, 0, 0))
        for c in range(NC):
            mx = scores(q0, c, mx)
        m_ref[...] = row_max(mx)

        def attn_fwd(b, pr):
            m = m_ref[...]
            outs = []
            for odd in range(2):
                h = 2 * pr + odd
                if odd:
                    nxt = _head(q_ref, jnp.minimum(b * NP + pr + 1, NB * NP - 1), 0)
                else:
                    nxt = _head(q_ref, b * NP + pr, 1)
                nxt = _as_weights(nxt)
                mx = acc = None
                for c in range(NC):
                    s = s_ref[keys(c), :].reshape(KC // 8, 8, BQ) - m[None]
                    p = jnp.exp2(s.reshape(KC, BQ))
                    for j in range(NL):
                        p_ref[h, j, keys(c), :] = p[:, j * 128:(j + 1) * 128].astype(BF)
                    mx = scores(nxt, c, mx)
                    r = _dot(vt_ref[:, keys(c)], p.astype(BF))
                    acc = r if acc is None else acc + r
                m = row_max(mx)
                inv = 1.0 / acc[DH:DH + 1]
                linv_ref[h] = jnp.broadcast_to(inv, (8, BQ))
                outs.append(acc * inv)
            m_ref[...] = m
            _store_pair(o_ref, pr, *outs)

        def attn_bwd(b, pr):
            skew = 2
            heads = []
            for odd in range(2):
                inv = linv_ref[2 * pr + odd]
                do = _rbf(_head(do_ref, pr, odd) * jnp.concatenate([inv] * (W // 8), axis=0))
                nd = -jnp.sum(do * _head(o_ref, pr, odd), axis=0, keepdims=True)
                hi = _rbf(nd)
                mid = _rbf(nd - hi)
                r = _rows((W, BQ))
                aug = jnp.where(r == DH, hi, jnp.where(r == DH + 1, mid,
                                jnp.where(r == DH + 2, nd - hi - mid, do)))
                heads.append((do, _as_weights(aug), _head(q_ref, b * NP + pr, odd)))
            ds, dq = {}, [None, None]
            for t in range(2 * NC + skew):
                if t < 2 * NC:
                    odd, c = divmod(t, NC)
                    do, dow, _ = heads[odd]
                    h = 2 * pr + odd
                    dp = _dot(v_ref[keys(c), :32], dow)
                    ds[t] = (dp * load_p(h, c, F32)).astype(BF)
                    dvt_ref[:, keys(c)] += _dot(do, load_p(h, c, BF), _NT)
                if t >= skew:
                    odd, c = divmod(t - skew, NC)
                    d = ds.pop(t - skew)
                    dkt_ref[:, keys(c)] += _dot(heads[odd][2], d, _NT)
                    r = _dot(kt_ref[:, keys(c)], d)
                    dq[odd] = r if dq[odd] is None else dq[odd] + r
            _store_pair(q_ref, b * NP + pr, dq[0] * SCALE, dq[1] * SCALE)

        def dense(b):
            ga, sb, cb1, gb = (_wide(mod_ref[j]) for j in range(2, 6))
            ob = o_ref[...].reshape(D, BQ).astype(BF)
            a = _dot(wo_ref[...], ob, _TN)
            gt = gin_ref[...].astype(F32).T
            df = (gt * gb).astype(BF)
            x1 = xt_ref[b].astype(F32) + ga * a
            n2, rstd2 = _normalize(x1)
            h2 = (n2 * cb1 + sb).astype(BF)
            ahead, dg = 2, {}
            for t in range(F // FC + ahead):
                if t < F // FC:
                    dg[t] = _dot(w2_ref[t * FC:(t + 1) * FC, :], df)
                if t >= ahead:
                    rows = slice((t - ahead) * FC, (t - ahead + 1) * FC)
                    u = _dot(w1t_ref[rows, :], h2)
                    sig = jax.nn.sigmoid(u)
                    act = u * sig
                    act_ref[rows, :] = act.astype(BF)
                    dact_ref[rows, :] = (dg.pop(t - ahead) * (sig + act * (1.0 - sig))).astype(BF)
            f = _dot(w2_ref[...], act_ref[...], _TN)
            ost_ref[...] = (x1 + gb * f).T.astype(BF)
            dmod_ref[5] += _fold(gt * f)
            dh2 = _dot(w1t_ref[...], dact_ref[...], _TN)
            dw2_ref[...] += _dot(act_ref[...], df, _NT)
            dmod_ref[3] += _fold(dh2)
            dmod_ref[4] += _fold(dh2 * n2)
            dx1 = gt + _normalize_bwd(dh2 * cb1, n2, rstd2)
            dx1_ref[b] = dx1
            dmod_ref[2] += _fold(dx1 * a)
            da = (dx1 * ga).astype(BF)
            do_ref[...] = _dot(wo_ref[...], da).reshape(NP, 2 * DH, BQ)
            dwo_ref[...] += _dot(ob, da, _NT)
            dw1t_ref[...] += _dot(dact_ref[...], h2, _NT)

        def block(b, carry):
            lax.fori_loop(0, NP, lambda pr, _: attn_fwd(b, pr), None)

            @pl.when(b == 0)
            def _():
                for cp in late:
                    cp.wait()

            @pl.when(b > 0)
            def _():
                out_copy(b - 1).wait()

            g_copy(b).wait()
            dense(b)
            out_copy(b).start()

            @pl.when(b + 1 < NB)
            def _():
                g_copy(b + 1).start()

            @pl.when(b + 1 == NB)
            def _():
                wo_ref[...] = dwo_ref[...].astype(BF)
                w1t_ref[...] = dw1t_ref[...].astype(BF)
                w2_ref[...] = dw2_ref[...].astype(BF)
                for cp in early_out:
                    cp.start()

            lax.fori_loop(0, NP, lambda pr, _: attn_bwd(b, pr), None)
            return carry

        lax.fori_loop(0, NB, block, 0)
        out_copy(NB - 1).wait()

    pl.run_scoped(main,
                  pltpu.VMEM((H, NL, S, 128), BF), pltpu.VMEM((S, BQ), F32), pltpu.VMEM((8, BQ), F32),
                  pltpu.VMEM((H, 8, BQ), F32),
                  pltpu.VMEM((NP, 2 * DH, BQ), F32), pltpu.VMEM((NP, 2 * DH, BQ), F32),
                  pltpu.VMEM((F, BQ), BF), pltpu.VMEM((F, BQ), BF), pltpu.VMEM((BQ, D), BF))

    def epilogue(wmod_ref, dwmod_ref, dxst_ref, h1_ref, dqb_ref, dkv_ref, dwq_ref, dwk_ref, dwv_ref, dc_ref):
        def dx_copy(b):
            rows = pl.ds(pl.multiple_of(b * BQ, BQ), BQ)
            return copy(dxst_ref.at[b], dx_hbm.at[rows], 4 + b)

        def dwmod_copy(lo, hi, i):
            return copy(dwmod_ref.at[:, lo * D:hi * D], dwmod_hbm.at[:, lo * D:hi * D], i)

        wmod_in = copy(wmod_hbm, wmod_ref, 8)
        wmod_in.start()
        c, sig, sc = silu_c()
        sc_col = jnp.concatenate([_to_col(sc)] * (D // 128), axis=1)

        def mod_grad(j):
            row = _rbf(_to_row(dmod_ref[j]))
            dwmod_ref[:, j * D:(j + 1) * D] = (sc_col * row).astype(BF)
            return row

        drows = [None, None] + [mod_grad(j) for j in range(2, 6)]
        dwmod_copy(2, 6, 9).start()
        valid = _rows((W, S)) < DH
        dkv_ref[...] = jnp.concatenate(
            [jnp.where(valid, dkt_ref[...] * LN2, 0.0), jnp.where(valid, dvt_ref[...], 0.0)],
            axis=0).astype(BF)

        def block(b, carry):
            cols = pl.ds(pl.multiple_of(b * BQ, BQ), BQ)
            dq = q_ref[pl.ds(b * NP, NP)].reshape(D, BQ).astype(BF)
            dqb_ref[:, cols] = dq
            dh1 = _dot(wq_ref[...], dq) + _dot(wkv_ref[...], dkv_ref[:, cols], _TN)
            ca1 = _wide(mod_ref[1])
            n1, rstd1 = _normalize(xt_ref[b].astype(F32))
            h1_ref[:, cols] = (n1 * ca1 + _wide(mod_ref[0])).astype(BF)
            dmod_ref[0] += _fold(dh1)
            dmod_ref[1] += _fold(dh1 * n1)
            dx = dx1_ref[b] + _normalize_bwd(dh1 * ca1, n1, rstd1)
            dxst_ref[b] = dx.T.astype(BF)
            dx_copy(b).start()
            return carry

        lax.fori_loop(0, NB, block, 0)
        drows[0], drows[1] = mod_grad(0), mod_grad(1)
        dwmod_copy(0, 2, 10).start()
        wmod_in.wait()
        dmod = jnp.broadcast_to(jnp.concatenate(drows, axis=1), (8, 6 * D))
        dsc = _dot(dmod, wmod_ref[...], _NT)[:1]
        dc_ref[...] = (dsc * (sig + c * sig * (1.0 - sig))).astype(BF)
        dwkv = _dot(dkv_ref[...], h1_ref[...], _NT)
        dwk_ref[...] = dwkv[:DH].astype(BF)
        dwv_ref[...] = dwkv[W:W + DH].astype(BF)
        last = [copy(dc_ref, dc_hbm, 11), copy(dwk_ref, dwkt_hbm, 12), copy(dwv_ref, dwvt_hbm, 13),
                copy(dwq_ref, dwq_hbm, 0)]
        dwq_ref[...] = _dot(h1_ref[...], dqb_ref[...], _NT).astype(BF)
        for cp in last:
            cp.start()
        for b in range(NB):
            dx_copy(b).wait()
        for cp in early_out + [dwmod_copy(2, 6, 9), dwmod_copy(0, 2, 10)] + last:
            cp.wait()

    pl.run_scoped(epilogue,
                  pltpu.VMEM((D, 6 * D), BF), pltpu.VMEM((D, 6 * D), BF), pltpu.VMEM((NB, BQ, D), BF),
                  pltpu.VMEM((D, S), BF), pltpu.VMEM((D, S), BF), pltpu.VMEM((2 * W, S), BF),
                  pltpu.VMEM((D, D), BF), pltpu.VMEM((DH, D), BF), pltpu.VMEM((DH, D), BF),
                  pltpu.VMEM((1, D), BF))


@jax.jit
def pallas_adaLN_cond__grouped_kv_mqa__dense_activation_silu__prompt_kernel(
    A_x: jax.Array,
    A_wq: jax.Array,
    A_wk: jax.Array,
    A_wv: jax.Array,
    A_wo: jax.Array,
    B_x: jax.Array,
    B_w1: jax.Array,
    B_w2: jax.Array,
    c: jax.Array,
    w_mod: jax.Array,
    grad_out: jax.Array,
):
    del B_x
    vmem = pltpu.VMEM
    shapes = [(S, D), (S, D), (D, D), (DH, D), (DH, D), (D, D), (F, D), (F, D), (1, D), (D, 6 * D)]
    out, dx, dwq, dwkt, dwvt, dwo, dw1t, dw2, dc, dwmod = pl.pallas_call(
        _kernel,
        out_shape=[jax.ShapeDtypeStruct(s, BF) for s in shapes],
        in_specs=[pl.BlockSpec(memory_space=pl.ANY)] * 10,
        out_specs=[pl.BlockSpec(memory_space=pl.ANY)] * 10,
        scratch_shapes=[
            vmem((NB, D, BQ), BF),
            vmem((NB * NP, 2 * DH, BQ), F32),
            vmem((NB, D, BQ), F32),
            vmem((S, 128), BF), vmem((S, 128), BF),
            vmem((W, S), F32), vmem((W, S), F32),
            vmem((W, S), F32), vmem((W, S), F32),
            vmem((D, D), BF), vmem((2 * W, D), BF), vmem((D, D), BF),
            vmem((F, D), BF), vmem((F, D), BF),
            vmem((1, D), BF),
            vmem((6, D, 128), F32), vmem((6, D, 128), F32),
            vmem((D, D), F32), vmem((F, D), F32), vmem((F, D), F32),
            vmem((BQ, D), BF),
            pltpu.SemaphoreType.DMA((14,)),
        ],
        compiler_params=pltpu.CompilerParams(vmem_limit_bytes=127 * 1024 * 1024),
        name="adaln_mqa_silu_fwd_bwd",
    )(A_x.reshape(S, D), A_wq, A_wk.T, A_wv.T, A_wo, B_w1.T, B_w2, c, w_mod, grad_out.reshape(S, D))
    return (out.reshape(1, S, D), dx.reshape(1, S, D), dwq, dwkt.T, dwvt.T, dwo, dw1t.T, dw2, dc, dwmod)
```

```python
import functools
import math

import jax
import jax.numpy as jnp
from jax import lax
import jax.experimental.pallas as pl
import jax.experimental.pallas.tpu as pltpu

S, D, H, DH, F = 2048, 640, 32, 20, 1728
BQ = 512
NB = S // BQ
NL = BQ // 128
UF, UB = 4, 4
LAG = 2
KC = 128
NC = S // KC
W = 24
WP = 32
FC = 256
FS = 64
VR = 16
RS = 32
QF = 256
SAFE_LOG2 = 48.0
EPS = 1e-5
SCALE = DH ** -0.5
LOG2E = math.log2(math.e)
LN2 = math.log(2.0)

BF, F32 = jnp.bfloat16, jnp.float32
_NN = (((1,), (0,)), ((), ()))
_NT = (((1,), (1,)), ((), ()))
_TN = (((0,), (0,)), ((), ()))


def _dot(a, b, dims=_NN):
    return lax.dot_general(a, b, dims, preferred_element_type=F32)


def _rows(shape):
    return lax.broadcasted_iota(jnp.int32, shape, 0)


def _rbf(x):
    return x.astype(BF).astype(F32)


def _wide(col):
    return jnp.concatenate([col] * NL, axis=1)


def _fold(x):
    acc = x[:, :128]
    for j in range(1, x.shape[1] // 128):
        acc = acc + x[:, j * 128:(j + 1) * 128]
    return acc


def _to_col(row):
    return jnp.broadcast_to(row, (128, D)).T


def _to_row(part):
    return jnp.sum(part.T, axis=0, keepdims=True)


def _strips(n=D, step=RS):
    return [slice(r, r + step) for r in range(0, n, step)]


def _add8(acc, x):
    part = jnp.sum(x.reshape(x.shape[0] // 8, 8, BQ), axis=0)
    return part if acc is None else acc + part


def _mean(acc):
    return jnp.sum(acc, axis=0, keepdims=True) * (1.0 / D)


def _moments(x):
    x = x.reshape(x.shape[0] // 8, 8, BQ)
    mean = jnp.sum(x, axis=0) * (1.0 / x.shape[0])
    xc = x - mean[None]
    return mean, jnp.sum(xc * xc, axis=0)


def _mean_rstd(groups):
    n = D // (8 * len(groups))
    mean = _mean(sum(m for m, _ in groups) * float(n))
    m2 = sum(q + float(n) * (m - mean) * (m - mean) for m, q in groups)
    return mean, lax.rsqrt(_mean(m2) + EPS)


def _zero(step):
    return lax.shift_right_logical(step, 10)


def _reread(rows, step):
    return pl.ds(pl.multiple_of(_zero(step) * 32 + rows.start, 32), rows.stop - rows.start)


def _aligned(start, n):
    return pl.ds(start if isinstance(start, int) else pl.multiple_of(start, n), n)


def _split_heads(x):
    keep = _rows((W, BQ)) < DH
    heads = []
    for lo in range(0, x.shape[0], 2 * DH):
        heads.append(jnp.where(keep, x[lo:lo + W], 0.0))
        heads.append(jnp.where(keep, pltpu.roll(x[lo + 2 * DH - W:lo + 2 * DH], DH, 0), 0.0))
    return heads


def _merge_heads(heads):
    parts = []
    for even, odd in zip(heads[::2], heads[1::2]):
        odd = pltpu.roll(odd, W - DH, 0)
        parts += [even[:16], jnp.where(_rows((8, BQ)) < 4, even[16:], odd[:8]), odd[8:]]
    return jnp.concatenate(parts, axis=0)


def _store_tiles(ref, idx, rows, x):
    for j in range(NL):
        ref[idx, j, rows, :] = x[:, j * 128:(j + 1) * 128].astype(BF)


def _load_tiles(ref, idx, rows):
    words = ref.bitcast(jnp.uint32)
    rows = slice(rows.start // 2, rows.stop // 2)
    return pltpu.bitcast(jnp.concatenate([words[idx, j, rows, :] for j in range(NL)], axis=1), BF)


def _fresh(ref, step, idx=0, deps=(), by_rows=False):
    words = ref.bitcast(jnp.uint32)
    tiles = [words[idx + _zero(step), j] for j in range(NL)]
    for j, dep in enumerate(deps):
        k, r = (0, 64 * (j + 1)) if by_rows else (j, 0)
        dep = lax.bitcast_convert_type(dep[-8:], jnp.uint32)
        held = _tie(tiles[k][r:r + 8], [dep[:, i:i + 128] for i in range(0, dep.shape[1], 128)], _true(step))
        tiles[k] = jnp.concatenate(([tiles[k][:r]] if r else []) + [held, tiles[k][r + 8:]], axis=0)
    return pltpu.bitcast(jnp.concatenate(tiles, axis=1), BF)


def _store_head(ref, idx, w):
    _store_tiles(ref, idx, slice(None), jnp.concatenate([w, jnp.zeros((WP - W, BQ), F32)], axis=0))


def _with_term(x, term):
    r = _rows((W, BQ))
    hi = _rbf(term)
    mid = _rbf(term - hi)
    return jnp.where(r == DH, hi, jnp.where(r == DH + 1, mid, jnp.where(r == DH + 2, term - hi - mid, x)))


class _VpuRows:
    def __init__(self, cols, rows, c, true):
        self.cols, self.rows, self.c, self.true, self.d, self.turn = cols, rows, c, true, 0, 0
        self.acc = lax.concatenate([rows[DH]] * (VR // 8), 0)

    def advance(self, upto):
        for d in range(self.d, upto):
            col = lax.concatenate([self.cols[self.c, d]] * NL, 1)
            self.acc = lax.add(self.acc, lax.mul(col, lax.concatenate([self.rows[d]] * (VR // 8), 0)))
        self.d = max(self.d, upto)

    def pace(self, x, plan):
        out = []
        for i in range(x.shape[0] // 8):
            xi = lax.slice_in_dim(x, 8 * i, 8 * i + 8)
            if i < len(plan) and plan[i] > self.d:
                self.advance(plan[i])
                r = self.turn % (VR // 8) * 8
                deps = lax.bitcast_convert_type(lax.slice_in_dim(self.acc, r, r + 8), x.dtype)
                xi = _tie(xi, [lax.slice_in_dim(deps, j * 128, (j + 1) * 128, axis=1) for j in range(NL)],
                          self.true)
                self.turn += 1
            out.append(xi)
        return lax.concatenate(out, 0)

    def result(self):
        self.advance(DH)
        return self.acc


def _true(step):
    return [_rows((8, 128)) + step >= -k for k in range(2)]


def _once(x, after, step):
    if after is None:
        return x
    return jnp.where(_rows((8, BQ)) + step >= 0, x, after[:8, :BQ])[:1]


def _tie(x, deps, true):
    first = lax.slice_in_dim(x, 0, 128, axis=1)
    for k, dep in enumerate(deps):
        first = lax.select(true[k % 2], first, dep)
    if x.shape[1] == 128:
        return first
    return lax.concatenate([first, lax.slice_in_dim(x, 128, x.shape[1], axis=1)], 1)


def _phases(x_hbm, wq_hbm, wkt_hbm, wvt_hbm, wo_hbm, w1t_hbm, w2_hbm, c_hbm, wmod_hbm, g_hbm,
            out_hbm, dx_hbm, dwq_hbm, dwkt_hbm, dwvt_hbm, dwo_hbm, dw1t_hbm, dw2_hbm, dc_hbm, dwmod_hbm,
            sem, xt_ref, q_ref, dq_ref, dx1_ref, k_ref, v_ref, kcol_ref, vcol_ref,
            kt_ref, vt_ref, dkt_ref, dvt_ref,
            wq_ref, wkv_buf, wo_buf, w12_ref, mod_ref, dmod_ref, stat_ref, scc_ref, dsilu_ref,
            dwo_ref, dw1t_ref, dw2_ref, dwo_st, dw12_st, io_ref, kvf_buf, kv_io, c_io,
            row_refs, lhs_ref, ds_refs, p_ref, o_ref, ob_ref, do_ref,
            a_ref, x1_ref, f_ref, dh2_ref, gt_ref, df_ref, h2_ref, da_ref, dkv_ref):
    w1t_ref, w2_ref, wkv_ref = w12_ref.at[0], w12_ref.at[1], wkv_buf.at[:2 * W]
    dw1t_st, dw2_st = dw12_st.at[0], dw12_st.at[1]
    wo_ref, gin_ref, ost_ref = wo_buf.at[0], io_ref.at[0], io_ref.at[1]
    wkvf_ref = dwkv_ref = kvf_buf.at[:2 * W]
    wk_ref, wv_ref, dwk_ref, dwv_ref = (kv_io.at[i] for i in range(4))
    c_ref, dc_ref = c_io.at[0], c_io.at[1]

    def copy(src, dst, i):
        return pltpu.make_async_copy(src, dst, sem.at[i])

    def tokens(b):
        return _aligned(b * BQ, BQ)

    def quarter(ref, b):
        return ref.at[b // 2, _aligned((b % 2) * D, D)]

    def g_copy(b):
        return copy(g_hbm.at[tokens(b)], gin_ref, 0)

    def wmod_cols(ref, lo, hi):
        return ref.at[:, lo * D:hi * D]

    late = [copy(wo_hbm, wo_ref, 1), copy(w1t_hbm, w1t_ref, 2), copy(w2_hbm, w2_ref, 3)]
    early_out = [copy(dwo_st, dwo_hbm, 1), copy(dw1t_st, dw1t_hbm, 2), copy(dw2_st, dw2_hbm, 3)]
    wmod_tail = [ref.at[i * D:(i + 1) * D] for ref in (w1t_ref, w2_ref) for i in range(2)]
    wmod_again = [copy(wmod_cols(wmod_hbm, 2 + i, 3 + i), wmod_tail[i], 14 + i) for i in range(4)]

    def silu_c():
        c = c_ref[...].astype(F32)
        sig = jax.nn.sigmoid(c)
        return c, sig, _rbf(c * sig)

    def accumulate(b, ref, staged, rows, lhs, rhs):
        total = jnp.where(b > 0, ref[rows, :], 0.0) + _dot(lhs, rhs, _NT)
        ref[rows, :] = total
        staged[rows, :] = total.astype(BF)
        return total

    def mod(j, rows):
        return _wide(mod_ref[j, rows, :])

    def prologue():
        xin_ref, wqt_ref, h1_ref = io_ref, dwo_st, df_ref

        def x_in(b):
            return copy(x_hbm.at[tokens(b)], xin_ref.at[b], 4 + b)

        def wmod_in(j, dst):
            cols = _aligned(j * D, D)
            return copy(wmod_hbm.at[:, cols], dst, 14 + j)

        first = [copy(c_hbm, c_ref, 8), wmod_in(0, wo_buf.at[0]), wmod_in(1, wo_buf.at[1]),
                 copy(wkt_hbm, wk_ref, 10), copy(wvt_hbm, wv_ref, 11), copy(wq_hbm, wq_ref, 12)]
        for cp in first + [x_in(0)]:
            cp.start()

        def statistics(b):
            groups = []
            for cols in _strips(step=128):
                xt = xin_ref[b, :, cols].T
                xt_ref[b, cols, :] = xt
                groups += [_moments(xt[r].astype(F32)) for r in _strips(128)]
            mean, rstd = _mean_rstd(groups)
            stat_ref[b, 0] = jnp.broadcast_to(mean, (8, BQ))
            stat_ref[b, 1] = jnp.broadcast_to(rstd, (8, BQ))

        def modulation(j, w):
            acc = 0.0
            for r in _strips():
                prod = w[r, :].astype(F32) * jnp.concatenate([scc_ref[r, :]] * (D // 128), axis=1)
                acc = acc + jnp.sum(prod.reshape(RS // 8, 8, D), axis=0)
            one = jnp.where((j == 1) | (j == 4), 1.0, 0.0)
            mod_ref[j] = _to_col(jnp.sum(acc, axis=0, keepdims=True) + one)

        def clear(j, carry):
            dmod_ref[j] = jnp.zeros((D, 128), F32)
            return carry

        lax.fori_loop(0, 6, clear, 0)
        for ref in (dkt_ref, dvt_ref, wkvf_ref):
            ref[...] = jnp.zeros(ref.shape, F32)
        o_ref[:UF] = jnp.zeros((UF, W, BQ), F32)
        p_ref[0, :, S - LAG * KC:, :] = jnp.zeros((NL, LAG * KC, 128), BF)
        for cp in first[:3]:
            cp.wait()
        c, sig, sc = silu_c()
        scc_ref[...] = _to_col(sc)
        dsilu_ref[:1, :] = sig + c * sig * (1.0 - sig)
        lax.fori_loop(0, 2, lambda j, _: modulation(j, wo_buf.at[j]), None)
        wmod_in(2, quarter(dw12_st, 0)).start()
        for cp in first[3:]:
            cp.wait()
        wqt_ref[...] = wq_ref[...].T
        wkvf_ref[:DH, :] = wk_ref[...].astype(F32)
        wkvf_ref[W:W + DH, :] = wv_ref[...].astype(F32)
        wkv_ref[...] = wkvf_ref[...].astype(BF)


        def block(b, carry):
            x_in(b).wait()

            @pl.when(b + 1 < NB)
            def _():
                x_in(b + 1).start()
                wmod_in(b + 3, quarter(dw12_st, b + 1)).start()

            statistics(b)
            wmod_in(b + 2, quarter(dw12_st, b)).wait()

            mean, rstd = stat_ref[b, 0, :1], stat_ref[b, 1, :1]
            for r in _strips():
                _store_tiles(h1_ref, 0, r, (xt_ref[b, r, :].astype(F32) - mean) * rstd * mod(1, r) + mod(0, r))
            modulation(b + 2, quarter(dw12_st, b))
            qt = [_dot(wqt_ref[:256, :], _load_tiles(h1_ref, 0, slice(0, D)))]
            kv = _rbf(_dot(wkv_ref[...], _fresh(h1_ref, b)))
            r = _rows((W, BQ))
            spare = (r >= DH) & (r < DH + 3)
            kt, vt = kv[:W], jnp.where(spare, 1.0, kv[W:])
            kt_ref[:, tokens(b)] = kt
            vt_ref[:, tokens(b)] = vt
            for src, ref, col_ref in ((jnp.where(spare, 1.0, kt), k_ref, kcol_ref), (vt, v_ref, vcol_ref)):
                rows = jnp.concatenate([src, jnp.zeros((128 - W, BQ), F32)], axis=0).T
                ref[tokens(b), :] = rows.astype(BF)
                for i in range(BQ // KC):
                    for d in range(DH):
                        col_ref[b * (BQ // KC) + i, d] = jnp.broadcast_to(
                            rows[(i + 1) * KC - VR:(i + 1) * KC, d:d + 1], (VR, 128))
            qt += [_dot(wqt_ref[r, :], _fresh(h1_ref, b + r.start)) for r in _strips(step=128)[2:]]
            qt = jnp.concatenate(qt, axis=0)
            q2, k2 = carry
            for h, q in enumerate(_split_heads(qt * (SCALE * LOG2E))):
                _store_head(q_ref, b * H + h, q)
                q2 = jnp.maximum(q2, jnp.sum(q * q, axis=0, keepdims=True))
            return q2, jnp.maximum(k2, jnp.sum(kt * kt, axis=0, keepdims=True))

        q2, k2 = lax.fori_loop(0, NB, block, (jnp.zeros((1, BQ), F32),) * 2)

        for cp in [g_copy(0)] + late:
            cp.start()

        @pl.when(jnp.logical_not(jnp.max(q2) * jnp.max(k2) <= SAFE_LOG2 ** 2))
        def _():
            def shift(h, carry):
                q = _load_tiles(q_ref, h, slice(0, WP))

                def chunk(c, mx):
                    s = _dot(k_ref[tokens(c), :WP], q)
                    return jnp.maximum(mx, jnp.max(s, axis=0, keepdims=True))

                mx = lax.fori_loop(0, NB, chunk, jnp.full((1, BQ), -jnp.inf, F32))
                _store_head(q_ref, h, _with_term(q.astype(F32)[:W], -mx))
                return carry

            lax.fori_loop(0, NB * H, shift, 0)

    prologue()

    def main():
        def out_copy(b):
            return copy(ost_ref, out_hbm.at[tokens(b)], 4)

        def keys(c):
            return slice(c * KC, (c + 1) * KC)

        def head(ref, h, dtype):
            return _load_tiles(ref, h, slice(0, WP)).astype(dtype)

        def spread(ref, h, slot, features=range(DH + 1)):
            x = head(ref, h, F32)
            for d in features:
                row = x[d:d + 1] if d < DH else x[DH:DH + 1] + x[DH + 1:DH + 2] + x[DH + 2:DH + 3]
                row_refs[slot][0, d] = jnp.broadcast_to(row, (8, BQ))

        def spread_next(x, ref, nxt, t, true):
            u, c = divmod(t, NC)
            if not 3 <= c < 3 + (DH + 1) // 3:
                return x
            spread(ref, nxt, (u + 1) % 2, range(3 * c - 9, 3 * c - 6))
            probe = row_refs[(u + 1) % 2][_zero(nxt), 3 * c - 7, :, BQ - 128:]
            return jnp.concatenate([x[:W - 8], _tie(x[W - 8:], [probe], true)], axis=0)

        def restart(r, i):
            return jnp.where(_rows(r.shape) + i >= 0, r, 0.0)

        def chunk_product(ref, c, w, mine, ahead, plan):
            lhs = ref.bitcast(jnp.uint32)[c * KC // 2:((c + 1) * KC - VR) // 2, :]
            out = _dot(pltpu.bitcast(ahead.pace(lhs, plan), BF)[:, :WP], w)
            return jnp.concatenate([out, mine], axis=0)

        def merged(i, n):
            rows = _aligned(i * n * DH, n * DH)
            return rows, _merge_heads([o_ref[i * n + u] for u in range(n)])

        def first_scores(b):
            spread(q_ref, b * H, 0)
            return _VpuRows(kcol_ref, row_refs[0].at[_zero(b)], 0, None).result()

        def attention_fwd(b, first):
            def values(h, c, lhs, acc, i, p=None):
                r = _dot(lhs, _load_tiles(p_ref, h, keys(c)) if p is None else p)
                acc = restart(r, i) if c == 0 else acc + r
                if c == NC - 1:
                    inv = 1.0 / acc[DH:DH + 1]
                    o_ref[h] = jnp.where(_rows((W, BQ)) == W - 1, inv, acc * inv)
                return acc

            def step(i, carry):
                mine, acc = carry
                true = _true(i)
                last = jnp.maximum(UF * i - 1, 0)
                early = [_load_tiles(p_ref, last, keys(c)) for c in range(NC - LAG, NC)]
                for t in range(UF * NC):
                    zero = _zero(i + t)
                    u, c = divmod(t, NC)
                    h = UF * i + u
                    ahead = _VpuRows(kcol_ref, row_refs[(t + 1) // NC % 2].at[zero], (t + 1) % NC, true)
                    s = chunk_product(k_ref, c, head(q_ref, b * H + h + zero, BF), mine, ahead,
                                      (2, 5, 7, 10, 12, 15, 17))
                    u1, c1 = divmod(t - LAG, NC)
                    lhs = spread_next(vt_ref[:, keys(c1)], q_ref,
                                      b * H + jnp.minimum(h + 1, H - 1) + zero, t, true)
                    acc = values(UF * i + u1 if t >= LAG else last, c1, ahead.pace(lhs, (DH,)), acc, i,
                                 None if t >= LAG else early[t])
                    _store_tiles(p_ref, h, keys(c), jnp.exp2(s))
                    mine = ahead.result()
                    if t == NC - 4:
                        rows, o = merged(jnp.maximum(i - 1, 0), UF)
                        _store_tiles(ob_ref, 0, rows, o)
                return mine, acc

            _, acc = lax.fori_loop(0, H // UF, step, (first, jnp.ones((W, BQ), F32)))

            @pl.when(b == 0)
            def _():
                for cp in late:
                    cp.wait()

            @pl.when(b > 0)
            def _():
                out_copy(b - 1).wait()

            g_copy(b).wait()
            for c in range(NC - LAG, NC):
                acc = values(H - 1, c, vt_ref[:, keys(c)], acc, b)
            rows, o = merged(H // UF - 1, UF)
            _store_tiles(ob_ref, 0, rows, o)

        def attention_bwd(b):
            def stage(h, slot):
                lhs_ref[slot, 0] = head(do_ref, h, F32)[:W]
                lhs_ref[slot, 1] = head(q_ref, b * H + h, F32)[:W]

            def grads(h, c, q, kt, acc, i):
                ds = ds_refs[c % len(ds_refs)]
                dkt_ref[:, keys(c)] += _dot(q, _load_tiles(ds, _zero(i), keys(0)), _NT)
                r = _dot(kt, _load_tiles(ds, _zero(i + 1), keys(0)))
                acc = restart(r, i) if c == 0 else acc + r
                if c == NC - 1:
                    o_ref[h] = acc * SCALE
                return acc

            def step(i, carry):
                mine, acc = carry
                true = _true(i)
                for t in range(UB * NC):
                    zero = _zero(i + t)
                    u, c = divmod(t, NC)
                    h = UB * i + u
                    nxt = jnp.minimum(h + 1, H - 1)
                    if c == NC - 4:
                        stage(nxt, (u + 1) % 2)
                    ahead = _VpuRows(vcol_ref, row_refs[(t + 1) // NC % 2].at[zero], (t + 1) % NC, true)
                    dp = chunk_product(v_ref, c, head(do_ref, h + zero, BF), mine, ahead,
                                       (2, 4, 6, 8, 10, 12, 14))
                    p = jnp.concatenate([p_ref[h, j, keys(c), :].astype(F32) for j in range(NL)], axis=1)
                    _store_tiles(ds_refs[c % len(ds_refs)], 0, slice(None), dp * p)
                    dvt_ref[:, keys(c)] += _dot(ahead.pace(lhs_ref[zero + u % 2, 0], (16,)),
                                                _load_tiles(p_ref, h, keys(c)), _NT)
                    u1, c1 = divmod(t - LAG, NC)
                    q = spread_next(lhs_ref[zero + u1 % 2, 1], do_ref, nxt + zero, t, true)
                    acc = grads(jnp.maximum(UB * i + u1, 0), c1, q,
                                ahead.pace(kt_ref[:, keys(c1)], (18, 0, DH)), acc, i + t)
                    mine = ahead.result()
                    if t == NC - 3:
                        rows, dq = merged(jnp.maximum(i - 1, 0), UB)
                        _store_tiles(dq_ref, b, rows, dq)
                return mine, acc

            stage(0, 0)
            lhs_ref[1, 1] = jnp.zeros((W, BQ), F32)
            for ref in ds_refs[-LAG:]:
                ref[...] = jnp.zeros(ref.shape, BF)
            spread(do_ref, 0, 0)
            first = _VpuRows(vcol_ref, row_refs[0].at[_zero(b)], 0, None).result()
            out_copy(b).start()

            @pl.when(b + 1 < NB)
            def _():
                g_copy(b + 1).start()

            @pl.when(b + 1 == NB)
            def _():
                for cp in early_out + wmod_again:
                    cp.start()

            _, acc = lax.fori_loop(0, H // UB, step, (first, jnp.zeros((W, BQ), F32)))
            for c in range(NC - LAG, NC):
                acc = grads(H - 1, c, lhs_ref[1, 1], kt_ref[:, keys(c)], acc, b)
            rows, dq = merged(H // UB - 1, UB)
            _store_tiles(dq_ref, b, rows, dq)

        def activation(u, dg):
            sig = 0.5 * jnp.tanh(0.5 * u) + 0.5
            act = u * sig
            return act.astype(BF), (dg * (sig + act * (1.0 - sig))).astype(BF)

        def mlp_chunk(j, b):
            lo = pl.multiple_of(j * FC, FC)
            parts = [activation(_dot(w1t_ref[pl.ds(lo + r, FS), :], _fresh(h2_ref, j + r)),
                                _dot(w2_ref[pl.ds(lo + r, FS), :], _fresh(df_ref, j + r)))
                     for r in range(0, FC, FS)]
            act, dact = (jnp.concatenate(p, axis=0) for p in zip(*parts))
            rows = pl.ds(lo, FC)
            accumulate(b, dw2_ref, dw2_st, rows, act, _fresh(df_ref, j + 1))
            accumulate(b, dw1t_ref, dw1t_st, rows, dact, _fresh(h2_ref, j + 1))
            f_ref[...] = jnp.where(j > 0, f_ref[...], 0.0) + _dot(w2_ref[rows, :], act, _TN)
            dh2_ref[...] = jnp.where(j > 0, dh2_ref[...], 0.0) + _dot(w1t_ref[rows, :], dact, _TN)
            return b

        def dense(b):
            groups = []
            for rows in _strips(step=128):
                a = _dot(wo_ref[:, rows], _fresh(ob_ref, b + rows.start), _TN)
                a_ref[rows, :] = a.astype(BF)
                x1 = xt_ref[b, rows, :].astype(F32) + mod(2, rows) * a
                x1_ref[rows, :] = x1
                groups.append(_moments(x1))
                gt = gin_ref[:, rows].T
                gt_ref[rows, :] = gt
                df = gt.astype(F32) * mod(5, rows)
                _store_tiles(df_ref, 0, rows, df)
            mean, rstd = _mean_rstd(groups)
            for r in _strips():
                _store_tiles(h2_ref, 0, r, (x1_ref[_reread(r, b), :] - mean) * rstd * mod(4, r) + mod(3, r))
            lo = F // FC * FC
            tail, mid = slice(lo, F), (lo + F) // 2
            dg = _dot(w2_ref[lo:mid, :], _fresh(df_ref, b))
            u = _dot(w1t_ref[tail, :], _load_tiles(h2_ref, 0, slice(0, D)))
            act, dact = activation(u, jnp.concatenate([dg, _dot(w2_ref[mid:, :], _fresh(df_ref, b + 1))], axis=0))

            lax.fori_loop(0, F // FC, mlp_chunk, b)

            n = mid - lo
            accumulate(b, dw2_ref, dw2_st, slice(lo, mid), act[:n], _fresh(df_ref, b + 2))
            s1 = s2 = None
            for r in _strips(step=128):
                dh2 = dh2_ref[r, :] + _dot(w1t_ref[tail, r], dact, _TN)
                dh2n = dh2 * ((x1_ref[r, :] - mean) * rstd)
                dmod_ref[3, r, :] += _fold(dh2)
                dmod_ref[4, r, :] += _fold(dh2n)
                dn = dh2 * mod(4, r)
                dh2_ref[r, :] = dn
                s1 = _add8(s1, dn)
                s2 = _add8(s2, dh2n * mod(4, r))
            s1, s2 = _mean(s1), _mean(s2) * rstd
            for r in _strips(step=128):
                f = f_ref[r, :] + _dot(w2_ref[tail, r], act, _TN)
                ost_ref[:, r] = (x1_ref[_reread(r, b), :] + mod(5, r) * f).astype(BF).T
                dmod_ref[5, r, :] += _fold(gt_ref[r, :].astype(F32) * f)
            done = []
            for r in _strips():
                rr = _reread(r, b + 1)
                dx1 = gt_ref[rr, :].astype(F32) + rstd * (dh2_ref[rr, :] - s1 - (x1_ref[rr, :] - mean) * s2)
                dx1_ref[b, r, :] = dx1
                _store_tiles(da_ref, 0, r, dx1 * mod(2, r))
                done.append(_fold(dx1 * a_ref[r, :].astype(F32)))
                dmod_ref[2, r, :] += done[-1]
            accumulate(b, dw2_ref, dw2_st, slice(mid, F), act[n:], _fresh(df_ref, b + 3, 0, done[1:8:2], True))
            accumulate(b, dw1t_ref, dw1t_st, slice(lo, mid), dact[:n], _fresh(h2_ref, b + 2, 0, done[8:15:2], True))
            accumulate(b, dw1t_ref, dw1t_st, slice(mid, F), dact[n:], _fresh(h2_ref, b + 3, 0, done[16:], True))

            def head_grads(g):
                done = []
                rows = pl.ds(pl.multiple_of(_zero(b) * 8 + 4 * DH * g, 8), 4 * DH)
                for h, do in enumerate(_split_heads(f_ref[rows, :]), 4 * g):
                    do = _rbf(do * o_ref[h, W - 1:])
                    done.append(_with_term(do, -jnp.sum(do * o_ref[h], axis=0, keepdims=True)))
                    _store_head(do_ref, h, done[-1])
                return done

            deps = []
            for i, rows in enumerate(_strips(step=128)):
                do = _dot(wo_ref[rows, :], _fresh(da_ref, b + i, deps=deps))
                deps = head_grads(i - 1) if i else []
                f_ref[rows, :] = do
            for i, rows in enumerate(_strips(step=128)):
                accumulate(b, dwo_ref, dwo_st, rows, _load_tiles(ob_ref, 0, rows),
                           _fresh(da_ref, b + i + 8, deps=deps, by_rows=True))
                deps = head_grads(i + 4) if i < 4 else []

        def block(b, first):
            attention_fwd(b, first)
            dense(b)
            attention_bwd(b)
            return first_scores(jnp.minimum(b + 1, NB - 1))

        lax.fori_loop(0, NB, block, first_scores(0))
        out_copy(NB - 1).wait()

    main()

    def epilogue():
        wmod_ref, dxst_ref, dh1_ref, dwq_ref = wo_buf, io_ref, dh2_ref, dwo_st

        def dx_out(b):
            return copy(dxst_ref.at[b], dx_hbm.at[tokens(b)], 4 + b)

        def dwmod_out(j, src):
            cols = _aligned(j * D, D)
            return copy(src, dwmod_hbm.at[:, cols], 18 + j)

        wmod_in = [copy(wmod_cols(wmod_hbm, j, j + 1), wmod_ref.at[j], 8 + j) for j in range(2)]
        for cp in wmod_in:
            cp.start()
        for cp in early_out + wmod_again:
            cp.wait()
        valid = _rows((W, S)) < DH
        dkv_ref[...] = jnp.concatenate(
            [jnp.where(valid, dkt_ref[...] * LN2, 0.0), jnp.where(valid, dvt_ref[...], 0.0)],
            axis=0).astype(BF)
        dw2_ref[:D, :128] = jnp.zeros((D, 128), F32)
        dwkv_ref[...] = jnp.zeros(dwkv_ref.shape, F32)

        pad = jnp.zeros((128 - 2 * W, D), F32)
        gt_ref[:, :128] = jnp.concatenate([wkv_ref[...].astype(F32), pad], axis=0).T.astype(BF)

        def mod_grad(j, w, dst):
            row = _rbf(_to_row(dmod_ref[j]))
            done = []
            for r in _strips():
                done.append(_fold(w[r, :].astype(F32) * row))
                dst[r, :] = (jnp.concatenate([scc_ref[r, :]] * (D // 128), axis=1) * row).astype(BF)
                dw2_ref[r, :128] += done[-1]
            return done

        def block(b, carry):
            mean, rstd = stat_ref[b, 0, :1], stat_ref[b, 1, :1]
            dkv = dkv_ref[:, tokens(b)]
            done = mod_grad(2 + b, quarter(w12_ref, b), quarter(dw12_st, b))
            s1 = s2 = None
            for i, r in enumerate(_strips(step=64)):
                w = jnp.concatenate([wq_ref[r, :], gt_ref[r, :2 * W]], axis=1)
                dh1 = _dot(w, jnp.concatenate(
                    [_fresh(dq_ref, b + i, b, done[max(3 * i - 6, 0):max(3 * i - 3, 0)]), dkv], axis=0))
                n1 = (xt_ref[b, r, :].astype(F32) - mean) * rstd
                _store_tiles(p_ref, b, r, n1 * mod(1, r) + mod(0, r))
                dh1n = dh1 * n1
                x1_ref[r, :128] += _fold(dh1)
                f_ref[r, :128] += _fold(dh1n)
                dn = dh1 * mod(1, r)
                dh1_ref[r, :] = dn
                s1 = _add8(s1, dn)
                s2 = _add8(s2, dh1n * mod(1, r))
            s1, s2 = _mean(s1), _mean(s2) * rstd
            def finish(i, after):
                r = slice(128 * i, 128 * i + 128)
                xc = xt_ref[b, _reread(r, b), :].astype(F32) - _once(mean, after, b)
                dx = dx1_ref[b, r, :] + rstd * (dh1_ref[_reread(r, b), :] - s1 - xc * s2)
                dxst_ref[b, :, r] = dx.astype(BF).T
                return [dx[q] for q in _strips(128, 32)]

            parts = finish(0, None)
            res = _dot(dkv, _load_tiles(p_ref, b + _zero(b), slice(0, D)), _NT)
            dwkv_ref[...] += res
            for i, r in enumerate(_strips(QF, 64)):
                nxt = finish(i + 1, res)
                res = accumulate(b, dwo_ref, dwq_ref, r, _load_tiles(p_ref, b + _zero(b + 1), r),
                                 _fresh(dq_ref, b + i + 16, b, parts, True))
                parts = nxt
            dx_out(b).start()
            dwmod_out(2 + b, quarter(dw12_st, b)).start()
            return b

        for ref in (x1_ref, f_ref):
            ref[:, :128] = jnp.zeros((D, 128), F32)
        lax.fori_loop(0, NB, block, 0)
        dmod_ref[0], dmod_ref[1] = x1_ref[:, :128], f_ref[:, :128]
        for cp in wmod_in:
            cp.wait()

        dwk_ref[...] = dwkv_ref[:DH, :].astype(BF)
        dwv_ref[...] = dwkv_ref[W:W + DH, :].astype(BF)
        last = [copy(dwk_ref, dwkt_hbm, 11), copy(dwv_ref, dwvt_hbm, 12),
                copy(dwq_ref.at[:QF], dwq_hbm.at[:QF], 13)]
        for cp in last:
            cp.start()

        def dwq_rows(rows, step, done=()):
            acc = 0.0
            for b in range(NB):
                h1 = jnp.concatenate([p_ref[b, k, rows, :] for k in range(NL)], axis=1)
                acc = acc + _dot(h1, _fresh(dq_ref, step, b, done[5 * b + 1:5 * b + 5], True), _NT)
            dwq_ref[rows, :] = acc.astype(BF)

        def tail(j, carry):
            dwq_rows(pl.ds(pl.multiple_of(QF + j * 128, 128), 128), j, mod_grad(j, wmod_ref.at[j], wmod_ref.at[j]))
            dwmod_out(j, wmod_ref.at[j]).start()
            return j

        step = lax.fori_loop(0, 2, tail, 0)
        dc_ref[...] = (_to_row(dw2_ref[:D, :128]) * dsilu_ref[:1, :]).astype(BF)
        dwq_rows(slice(QF + 256, D), step)
        last += [copy(dwq_ref.at[QF:], dwq_hbm.at[QF:], 0), copy(dc_ref, dc_hbm, 10)]
        for cp in last[-2:]:
            cp.start()
        last += [dwmod_out(j, wmod_ref.at[j]) for j in range(2)]
        last += [dwmod_out(2 + b, quarter(dw12_st, b)) for b in range(NB)]
        for cp in [dx_out(b) for b in range(NB)] + last:
            cp.wait()

    epilogue()


def _kernel(*refs):
    vmem = pltpu.VMEM
    pl.run_scoped(
        functools.partial(_phases, *refs),
        vmem((NB, D, BQ), BF),
        vmem((NB * H, NL, WP, 128), BF),
        vmem((NB, NL, D, 128), BF),
        vmem((NB, D, BQ), F32),
        vmem((S, 128), BF), vmem((S, 128), BF),
        vmem((NC, DH, VR, 128), F32), vmem((NC, DH, VR, 128), F32),
        vmem((W, S), F32), vmem((W, S), F32),
        vmem((W, S), F32), vmem((W, S), F32),
        vmem((D, D), BF), vmem((64, D), BF), vmem((2, D, D), BF),
        vmem((2, F, D), BF),
        vmem((6, D, 128), F32), vmem((6, D, 128), F32),
        vmem((NB, 2, 8, BQ), F32),
        vmem((D, 128), F32), vmem((32, D), F32),
        vmem((D, D), F32), vmem((F, D), F32), vmem((F, D), F32),
        vmem((D, D), BF), vmem((2, F, D), BF),
        vmem((NB, BQ, D), BF),
        vmem((64, D), F32), vmem((8, DH, D), BF), vmem((32, 1, D), BF),
        [vmem((1, DH + 1, 8, BQ), F32)] * 2,
        vmem((2, 2, W, BQ), F32),
        [vmem((1, NL, KC, 128), BF)] * 4,
        vmem((H, NL, S, 128), BF),
        vmem((H, W, BQ), F32), vmem((1, NL, D, 128), BF),
        vmem((H, NL, WP, 128), BF),
        vmem((D, BQ), BF), vmem((D, BQ), F32), vmem((D, BQ), F32), vmem((D, BQ), F32), vmem((D, BQ), BF),
        vmem((1, NL, D, 128), BF), vmem((1, NL, D, 128), BF), vmem((1, NL, D, 128), BF),
        vmem((2 * W, S), BF),
    )


@jax.jit
def pallas_adaLN_cond__grouped_kv_mqa__dense_activation_silu__prompt_kernel(
    A_x: jax.Array,
    A_wq: jax.Array,
    A_wk: jax.Array,
    A_wv: jax.Array,
    A_wo: jax.Array,
    B_x: jax.Array,
    B_w1: jax.Array,
    B_w2: jax.Array,
    c: jax.Array,
    w_mod: jax.Array,
    grad_out: jax.Array,
):
    del B_x
    shapes = [(S, D), (S, D), (D, D), (DH, D), (DH, D), (D, D), (F, D), (F, D), (1, D), (D, 6 * D)]
    out, dx, dwq, dwkt, dwvt, dwo, dw1t, dw2, dc, dwmod = pl.pallas_call(
        _kernel,
        out_shape=[jax.ShapeDtypeStruct(s, BF) for s in shapes],
        in_specs=[pl.BlockSpec(memory_space=pl.ANY)] * 10,
        out_specs=[pl.BlockSpec(memory_space=pl.ANY)] * 10,
        scratch_shapes=[pltpu.SemaphoreType.DMA((24,))],
        compiler_params=pltpu.CompilerParams(vmem_limit_bytes=128 * 1024 * 1024),
        name="adaln_mqa_silu_fwd_bwd",
    )(A_x.reshape(S, D), A_wq, A_wk.T, A_wv.T, A_wo, B_w1.T, B_w2, c, w_mod, grad_out.reshape(S, D))
    return (out.reshape(1, S, D), dx.reshape(1, S, D), dwq, dwkt.T, dwvt.T, dwo, dw1t.T, dw2, dc, dwmod)
```
